```python
import jax
import jax.numpy as jnp

def _softmax(x, axis=-1):
    return jax.nn.softmax(x, axis=axis)
def _gelu(x):
    return jax.nn.gelu(x, approximate=True)
def _silu(x):
    return jax.nn.silu(x)
def _sigmoid(x):
    return jax.nn.sigmoid(x)
def _layernorm(x, axis=-1, eps=1e-5):
    m = jnp.mean(x, axis=axis, keepdims=True)
    v = jnp.var(x, axis=axis, keepdims=True)
    return (x - m) / jnp.sqrt(v + eps)
def _scatter_add(tgt, idx, src, axis=0):
    return tgt.at[idx].add(src)
def _segment_sum(src, seg, n):
    return jax.ops.segment_sum(src, seg, n)
class _Rng:
    def __init__(self, key):
        self._k = key
    def _next(self):
        self._k, sub = jax.random.split(self._k)
        return sub
    def normal(self, shape):
        return jax.random.normal(self._next(), shape, dtype=jnp.bfloat16)
    def randint(self, lo, hi, shape):
        return jax.random.randint(self._next(), shape, lo, hi, dtype=jnp.int32)
    def uniform(self, shape, lo=0.0, hi=1.0):
        return jax.random.uniform(self._next(), shape, jnp.bfloat16, lo, hi)
    def permutation(self, n):
        return jax.random.permutation(self._next(), n)


kernel_name = 'gated_mix__compressed_kv_cla__ssm_conv_h3__prompt'

def setup_inputs():
    _rng = _Rng(jax.random.key(int.from_bytes(__import__("os").urandom(4), "little")))
    _w = (lambda a: (lambda t: t.astype(jnp.bfloat16) if jnp.issubdtype(t.dtype, jnp.floating) else t)(jnp.asarray(a)))
    def _A_setup():
        B, H, Sq, Sk, D, M = 1, 32, 2048, 2048, 128, 1024
        Dc = 4 * D
        return {
            "x": _w((lambda *s: _rng.normal(s) * 0.05)(B, Sq, M)),
            "c_kv": _w((lambda *s: _rng.normal(s) * 0.05)(B, Sk, Dc)),
            "w_q": _w((lambda *s: _rng.normal(s) * 0.05)(M, H, D) * (M ** -0.5)),
            "w_uk": _w((lambda *s: _rng.normal(s) * 0.05)(Dc, H, D) * (Dc ** -0.5)),
            "w_uv": _w((lambda *s: _rng.normal(s) * 0.05)(Dc, H, D) * (Dc ** -0.5)),
            "w_o": _w((lambda *s: _rng.normal(s) * 0.05)(H, D, M) * ((H * D) ** -0.5)),
        }
    _A_in = _A_setup()

    def _B_setup():
        B, S, D = 1, 2048, 1024
        ks = 4
        return {
            "q": _w((lambda *s: _rng.normal(s) * 0.05)(B, S, D)),
            "k": _w((lambda *s: _rng.normal(s) * 0.05)(B, S, D)),
            "v": _w((lambda *s: _rng.normal(s) * 0.05)(B, S, D)),
            "shift_k": _w((lambda *s: _rng.normal(s) * 0.05)(D, ks) * 0.5),
            "ssm_k": _w((lambda *s: _rng.normal(s) * 0.05)(D, S) * (1.0 / S ** 0.5)),
            "ssm_D": _w((lambda *s: _rng.normal(s) * 0.05)(D)),
        }
    _B_in = _B_setup()

    return {
        "A_x": _A_in["x"],
        "A_c_kv": _A_in["c_kv"],
        "A_w_q": _A_in["w_q"],
        "A_w_uk": _A_in["w_uk"],
        "A_w_uv": _A_in["w_uv"],
        "A_w_o": _A_in["w_o"],
        "B_q": _B_in["q"],
        "B_k": _B_in["k"],
        "B_v": _B_in["v"],
        "B_shift_k": _B_in["shift_k"],
        "B_ssm_k": _B_in["ssm_k"],
        "B_ssm_D": _B_in["ssm_D"],
        "gate_w": _w((lambda *s: _rng.normal(s) * 0.05)(1024)),
    }

def reference(A_x, A_c_kv, A_w_q, A_w_uk, A_w_uv, A_w_o, B_q, B_k, B_v, B_shift_k, B_ssm_k, B_ssm_D, gate_w):
    def _A_ref(x, c_kv, w_q, w_uk, w_uv, w_o):
        B, Sq, M = x.shape[0], x.shape[1], x.shape[2]
        Sk = c_kv.shape[1]
        H, D = w_q.shape[1], w_q.shape[2]
        q = jnp.einsum("bqm,mhd->bhqd", x, w_q)
        k = jnp.einsum("bkc,chd->bhkd", c_kv, w_uk)
        v = jnp.einsum("bkc,chd->bhkd", c_kv, w_uv)
        scores = jnp.einsum("bhqd,bhkd->bhqk", q, k) * (D ** -0.5)
        off = Sk - Sq
        qi = jnp.arange(Sq)[:, None]
        kj = jnp.arange(Sk)[None, :]
        cmask = kj <= (qi + off)
        scores = jnp.where(cmask[None, None], scores, -1e9)
        p = _softmax(scores, axis=-1)
        ctx = jnp.einsum("bhqk,bhkd->bhqd", p, v)
        return jnp.einsum("bhqd,hdm->bqm", ctx, w_o)

    def _B_ref(q, k, v, shift_k, ssm_k, ssm_D):
        B, S, D = q.shape
        ks = shift_k.shape[-1]
        k_pad = jnp.pad(k, ((0, 0), (ks - 1, 0), (0, 0)))
        k_shift = jnp.zeros_like(k)
        for t in range(ks):
            k_shift = k_shift + k_pad[:, t:t + S, :] * shift_k[:, ks - 1 - t][None, None, :]
        kv = k_shift * v
        L = 2 * S
        kv_pad = jnp.pad(kv, ((0, 0), (0, S), (0, 0)))
        kf_pad = jnp.pad(ssm_k, ((0, 0), (0, S)))
        kv_f = (lambda x, axes=(-2,-1): jnp.fft.rfft2(x.astype(jnp.float32), axes=axes))(kv_pad[:, None, :, :], axes=(1, 2))
        kf_f = (lambda x, axes=(-2,-1): jnp.fft.rfft2(x.astype(jnp.float32), axes=axes))(kf_pad[:, None, :], axes=(1, 2))
        kf_f = (lambda x, *d: x.transpose(*d))(kf_f, 1, 2, 0)
        y_f = kv_f * kf_f[None, :, :, :]
        y = (lambda x, s, axes=(-2,-1): jnp.fft.irfft2(x, s=s, axes=axes).astype(jnp.bfloat16))(y_f, (1, L), axes=(1, 2))[:, 0, :S, :]
        y = y + kv * ssm_D[None, None, :]
        return q * y

    x = A_x
    g = _sigmoid((x * gate_w).sum(-1, keepdims=True))
    a = _A_ref(x, A_c_kv, A_w_q, A_w_uk, A_w_uv, A_w_o)
    b = _B_ref(x, B_k, B_v, B_shift_k, B_ssm_k, B_ssm_D)
    return g * a + (1 - g) * b
```

```python
import math
import numpy as np
import jax
import jax.numpy as jnp
import jax.experimental.pallas as pl
import jax.experimental.pallas.tpu as pltpu

S = 2048
M = 1024
H = 32
D = 128
DC = 512
BQ = 2048
T = 128
NI = S // T
NO = 4
HP = 1
NS = H // HP
BF = jnp.bfloat16
F32 = jnp.float32
NEG = -1e30


def _dft_consts():
    k = np.arange(T)[:, None] + 0.5
    a = np.arange(T)[None, :]
    th = 2 * np.pi * k * a / (2 * T)
    fwd = np.concatenate([np.cos(th), -np.sin(th)], 0)
    n = np.arange(2 * T)[:, None]
    th2 = 2 * np.pi * k.T * n / (2 * T)
    inv = np.concatenate([np.cos(th2), -np.sin(th2)], 1) / T
    inv2 = np.concatenate([inv[:T], inv[T:]], 1)
    return fwd.astype(np.float32), inv2.astype(np.float32)


def _nt(a, b):
    return jax.lax.dot_general(a, b, (((1,), (1,)), ((), ())), preferred_element_type=F32)


def _mm(a, b):
    return jnp.dot(a, b, preferred_element_type=F32)


def _kernel(x_ref, c_ref, wq_ref, wuk_ref, wuv_ref, wo_hbm, bk_ref, bv_ref, sk_ref,
            f_ref, dd_ref, gw_ref, fwd_ref, inv_ref, o_ref,
            ctx_s, b_s, wo_s, u_s, uf_s, ff_s, y_s, sem):
    step = pl.program_id(0)
    wo_copy = pltpu.make_async_copy(wo_hbm, wo_s, sem)

    @pl.when(step == 0)
    def _():
        wo_copy.start()

    per = NS // 8

    @pl.when(jnp.logical_and(step % per == 0, step < NS))
    def _():
        with jax.named_scope("ssm"):
            kk = bk_ref[...].astype(F32)
            row = jax.lax.broadcasted_iota(jnp.int32, (S, T), 0)
            sk = sk_ref[...].astype(F32)
            acc = kk * sk[0:1]
            for t in range(1, 4):
                sh = jnp.where(row >= t, pltpu.roll(kk, t, 0), 0.0)
                acc = acc + sh * sk[t:t + 1]
            kv = acc.astype(BF) * bv_ref[...]
            u_s[...] = kv
            fwd = fwd_ref[...]
            for i in range(NI):
                uf_s[i] = _mm(fwd, u_s[i * T:(i + 1) * T, :])
                ff_s[i] = _nt(fwd, f_ref[:, i * T:(i + 1) * T])

            def body(r, carry):
                r0 = pl.multiple_of(r * 16, 16)
                ra = pl.ds(r0, 16)
                rb = pl.ds(r0 + T, 16)
                for i in range(NI):
                    yr = None
                    for j in range(i + 1):
                        ua, ub = uf_s[j, ra, :], uf_s[j, rb, :]
                        fa, fb = ff_s[i - j, ra, :], ff_s[i - j, rb, :]
                        tr = ua * fa - ub * fb
                        ti = ua * fb + ub * fa
                        yr, yi = (tr, ti) if yr is None else (yr + tr, yi + ti)
                    y_s[i + 1, ra, :] = yr.astype(BF)
                    y_s[i + 1, rb, :] = yi.astype(BF)
                return carry
            jax.lax.fori_loop(0, T // 16, body, 0)
            y_s[0] = jnp.zeros((2 * T, T), BF)
            inv = inv_ref[...]
            dd = dd_ref[...].astype(F32)
            c0 = pl.multiple_of((step // per) * T, T)
            for i in range(NI):
                y = _mm(inv[:, :2 * T], y_s[i + 1]) + _mm(inv[:, 2 * T:], y_s[i])
                y = y + u_s[i * T:(i + 1) * T, :].astype(F32) * dd
                b_s[i * T:(i + 1) * T, pl.ds(c0, T)] = y

    @pl.when(step < NS)
    def _():
        x = x_ref[...]
        c = c_ref[...]
        qa = (_mm(x, wq_ref[...]) * (D ** -0.5 * math.log2(math.e))).astype(BF)
        ka = _mm(c, wuk_ref[...]).astype(BF)
        va = _mm(c, wuv_ref[...]).astype(BF)
        tri = (jax.lax.broadcasted_iota(jnp.int32, (T, T), 1)
               <= jax.lax.broadcasted_iota(jnp.int32, (T, T), 0))
        nd = BQ // T
        for hh in range(HP):
            q = qa[:, hh * D:(hh + 1) * D]
            k = ka[:, hh * D:(hh + 1) * D]
            v = va[:, hh * D:(hh + 1) * D]
            for I in range(S // BQ):
                base = I * BQ
                qb = q[base:base + BQ]
                parts = [(0, a, 256) for a in range(0, base, 256)]
                parts += [(j * T, base + j * T, T) for j in range(nd)]
                ss = []
                for idx, (r0, k0, kl) in enumerate(parts):
                    s = _nt(qb[r0:], k[k0:k0 + kl])
                    if k0 >= base:
                        top = jnp.where(tri, s[:T], NEG)
                        s = top if r0 + T == BQ else jnp.concatenate([top, s[T:]], 0)
                    ss.append(s)

                def rowred(op, vals, red):
                    outs = []
                    for r in range(nd):
                        m = None
                        for (r0, k0, kl), s in zip(parts, vals):
                            if r0 <= r * T:
                                blk = s[r * T - r0:(r + 1) * T - r0]
                                for t in range(kl // T):
                                    e = blk[:, t * T:(t + 1) * T]
                                    m = e if m is None else op(m, e)
                        outs.append(red(m, axis=1, keepdims=True))
                    return jnp.concatenate(outs, 0)
                m = rowred(jnp.maximum, ss, jnp.max)
                ps = [jnp.exp2(s - m[r0:]) for (r0, _, _), s in zip(parts, ss)]
                l = rowred(jnp.add, ps, jnp.sum)
                acc = None
                cur = 0
                done = []
                for (r0, k0, kl), p in zip(parts, ps):
                    if r0 > cur:
                        done.append(acc[:T])
                        acc = acc[T:]
                        cur = r0
                    pv = _mm(p.astype(BF), v[k0:k0 + kl])
                    acc = pv if acc is None else acc + pv
                done.append(acc)
                o = jnp.concatenate(done, 0) * (1.0 / l)
                c0 = pl.multiple_of((step * HP + hh) * D, D)
                ctx_s[base:base + BQ, pl.ds(c0, D)] = o.astype(BF)

    @pl.when(step == NS)
    def _():
        wo_copy.wait()

    @pl.when(step >= NS)
    def _():
        R = S // NO
        r0 = pl.multiple_of((step - NS) * R, R)
        rs = pl.ds(r0, R)
        a = _mm(ctx_s[rs, :], wo_s[...])
        xb = x_ref[rs, :]
        z = jnp.sum((xb * gw_ref[...]).astype(F32), axis=1, keepdims=True)
        g = jax.nn.sigmoid(z)
        b = xb.astype(F32) * b_s[rs, :]
        o_ref[...] = (g * a + (1.0 - g) * b).astype(o_ref.dtype)


@jax.jit
def pallas_gated_mix__compressed_kv_cla__ssm_conv_h3__prompt_kernel(
    A_x, A_c_kv, A_w_q, A_w_uk, A_w_uv, A_w_o, B_q, B_k, B_v, B_shift_k,
    B_ssm_k, B_ssm_D, gate_w,
):
    fwd, inv = _dft_consts()
    per = NS // 8
    hm = lambda s: (0, jnp.minimum(s, NS - 1))
    cm = lambda s: (0, jnp.minimum(s // per, 7))
    full = lambda shape: pl.BlockSpec(shape, lambda s: (0, 0))
    out = pl.pallas_call(
        _kernel,
        grid=(NS + NO,),
        in_specs=[
            full((S, M)), full((S, DC)),
            pl.BlockSpec((M, HP * D), hm),
            pl.BlockSpec((DC, HP * D), hm),
            pl.BlockSpec((DC, HP * D), hm),
            pl.BlockSpec(memory_space=pl.ANY),
            pl.BlockSpec((S, T), cm), pl.BlockSpec((S, T), cm),
            pl.BlockSpec((4, T), cm),
            pl.BlockSpec((T, S), lambda s: (jnp.minimum(s // per, 7), 0)),
            pl.BlockSpec((1, T), cm),
            full((1, M)), full((2 * T, T)), full((T, 4 * T)),
        ],
        out_specs=pl.BlockSpec((S // NO, M), lambda s: (jnp.maximum(s - NS, 0), 0)),
        out_shape=jax.ShapeDtypeStruct((S, M), A_x.dtype),
        scratch_shapes=[
            pltpu.VMEM((S, H * D), BF), pltpu.VMEM((S, M), F32), pltpu.VMEM((H * D, M), BF),
            pltpu.VMEM((S, T), BF), pltpu.VMEM((NI, 2 * T, T), F32),
            pltpu.VMEM((NI, 2 * T, T), F32), pltpu.VMEM((NI + 1, 2 * T, T), BF),
            pltpu.SemaphoreType.DMA(()),
        ],
        compiler_params=pltpu.CompilerParams(
            dimension_semantics=("arbitrary",), vmem_limit_bytes=110 * 1024 * 1024),
    )(A_x[0], A_c_kv[0], A_w_q.reshape(M, H * D), A_w_uk.reshape(DC, H * D),
      A_w_uv.reshape(DC, H * D), A_w_o.reshape(H * D, M), B_k[0], B_v[0], B_shift_k.T,
      B_ssm_k, B_ssm_D.reshape(1, M), gate_w.reshape(1, M),
      jnp.asarray(fwd, BF), jnp.asarray(inv, BF))
    return out[None]
```

```python
import math
import numpy as np
import jax
import jax.numpy as jnp
import jax.experimental.pallas as pl
import jax.experimental.pallas.tpu as pltpu

S = 2048
M = 1024
H = 32
D = 128
DC = 512
BQ = 2048
T = 128
NI = S // T
NO = 4
HP = 1
NS = H // HP
BF = jnp.bfloat16
F32 = jnp.float32
NEG = -1e30


def _dft_consts():
    k = np.arange(T)[:, None] + 0.5
    a = np.arange(T)[None, :]
    th = 2 * np.pi * k * a / (2 * T)
    fwd = np.concatenate([np.cos(th), -np.sin(th)], 0)
    n = np.arange(2 * T)[:, None]
    th2 = 2 * np.pi * k.T * n / (2 * T)
    inv = np.concatenate([np.cos(th2), -np.sin(th2)], 1) / T
    inv2 = np.concatenate([inv[:T], inv[T:]], 1)
    return fwd.astype(np.float32), inv2.astype(np.float32)


def _nt(a, b):
    return jax.lax.dot_general(a, b, (((1,), (1,)), ((), ())), preferred_element_type=F32)


def _mm(a, b):
    return jnp.dot(a, b, preferred_element_type=F32)


def _kernel(x_ref, c_ref, wq_ref, wuk_ref, wuv_ref, wo_hbm, bk_ref, bv_ref, sk_ref,
            f_ref, dd_ref, gw_ref, fwd_ref, inv_ref, o_ref,
            ctx_s, b_s, wo_s, u_s, uf_s, ff_s, y_s, sem, wq_s, wk_s, wv_s, wsem):
    step = pl.program_id(0)
    wo_copy = pltpu.make_async_copy(wo_hbm, wo_s, sem)

    def wcopies(h):
        return [pltpu.make_async_copy(w.bitcast(jnp.uint32).at[:, h // 2, :],
                                      b.at[h % 2], wsem.at[i, h % 2])
                for i, (w, b) in enumerate(((wq_ref, wq_s), (wuk_ref, wk_s), (wuv_ref, wv_s)))]

    def getw(b):
        sh = (16 * (1 - step % 2)).astype(jnp.uint32)
        bits = (b[step % 2] << sh) & jnp.uint32(0xFFFF0000)
        return pltpu.bitcast(bits, F32).astype(BF)

    @pl.when(step == 0)
    def _():
        for cp in wcopies(step):
            cp.start()
        wo_copy.start()

    @pl.when(step < NS)
    def _():
        for cp in wcopies(step):
            cp.wait()

        @pl.when(step + 1 < NS)
        def _():
            for cp in wcopies(step + 1):
                cp.start()

    per = NS // 8

    @pl.when(jnp.logical_and(step % per == 0, step < NS))
    def _():
        with jax.named_scope("ssm"):
            kk = bk_ref[...].astype(F32)
            row = jax.lax.broadcasted_iota(jnp.int32, (S, T), 0)
            sk = sk_ref[...].astype(F32)
            acc = kk * sk[0:1]
            for t in range(1, 4):
                sh = jnp.where(row >= t, pltpu.roll(kk, t, 0), 0.0)
                acc = acc + sh * sk[t:t + 1]
            kv = acc.astype(BF) * bv_ref[...]
            u_s[...] = kv
            fwd = fwd_ref[...]
            for i in range(NI):
                uf_s[i] = _mm(fwd, u_s[i * T:(i + 1) * T, :])
                ff_s[i] = _nt(fwd, f_ref[:, i * T:(i + 1) * T])

            def body(r, carry):
                r0 = pl.multiple_of(r * 16, 16)
                ra = pl.ds(r0, 16)
                rb = pl.ds(r0 + T, 16)
                for i in range(NI):
                    yr = None
                    for j in range(i + 1):
                        ua, ub = uf_s[j, ra, :], uf_s[j, rb, :]
                        fa, fb = ff_s[i - j, ra, :], ff_s[i - j, rb, :]
                        tr = ua * fa - ub * fb
                        ti = ua * fb + ub * fa
                        yr, yi = (tr, ti) if yr is None else (yr + tr, yi + ti)
                    y_s[i + 1, ra, :] = yr.astype(BF)
                    y_s[i + 1, rb, :] = yi.astype(BF)
                return carry
            jax.lax.fori_loop(0, T // 16, body, 0)
            y_s[0] = jnp.zeros((2 * T, T), BF)
            inv = inv_ref[...]
            dd = dd_ref[...].astype(F32)
            c0 = pl.multiple_of((step // per) * T, T)
            for i in range(NI):
                y = _mm(inv[:, :2 * T], y_s[i + 1]) + _mm(inv[:, 2 * T:], y_s[i])
                y = y + u_s[i * T:(i + 1) * T, :].astype(F32) * dd
                b_s[i * T:(i + 1) * T, pl.ds(c0, T)] = y

    @pl.when(step < NS)
    def _():
        x = x_ref[...]
        c = c_ref[...]
        qa = (_mm(x, getw(wq_s)) * (D ** -0.5 * math.log2(math.e))).astype(BF)
        ka = _mm(c, getw(wk_s)).astype(BF)
        va = _mm(c, getw(wv_s)).astype(BF)
        tri = (jax.lax.broadcasted_iota(jnp.int32, (T, T), 1)
               <= jax.lax.broadcasted_iota(jnp.int32, (T, T), 0))
        nd = BQ // T
        for hh in range(HP):
            q = qa[:, hh * D:(hh + 1) * D]
            k = ka[:, hh * D:(hh + 1) * D]
            v = va[:, hh * D:(hh + 1) * D]
            for I in range(S // BQ):
                base = I * BQ
                qb = q[base:base + BQ]
                parts = [(0, a, 256) for a in range(0, base, 256)]
                parts += [(j * T, base + j * T, T) for j in range(nd)]
                ss = []
                for idx, (r0, k0, kl) in enumerate(parts):
                    s = _nt(qb[r0:], k[k0:k0 + kl])
                    if k0 >= base:
                        top = jnp.where(tri, s[:T], NEG)
                        s = top if r0 + T == BQ else jnp.concatenate([top, s[T:]], 0)
                    ss.append(s)

                def rowred(op, vals, red):
                    outs = []
                    for r in range(nd):
                        m = None
                        for (r0, k0, kl), s in zip(parts, vals):
                            if r0 <= r * T:
                                blk = s[r * T - r0:(r + 1) * T - r0]
                                for t in range(kl // T):
                                    e = blk[:, t * T:(t + 1) * T]
                                    m = e if m is None else op(m, e)
                        outs.append(red(m, axis=1, keepdims=True))
                    return jnp.concatenate(outs, 0)
                m = rowred(jnp.maximum, ss, jnp.max)
                ps = [jnp.exp2(s - m[r0:]) for (r0, _, _), s in zip(parts, ss)]
                l = rowred(jnp.add, ps, jnp.sum)
                acc = None
                cur = 0
                done = []
                for (r0, k0, kl), p in zip(parts, ps):
                    if r0 > cur:
                        done.append(acc[:T])
                        acc = acc[T:]
                        cur = r0
                    pv = _mm(p.astype(BF), v[k0:k0 + kl])
                    acc = pv if acc is None else acc + pv
                done.append(acc)
                o = jnp.concatenate(done, 0) * (1.0 / l)
                c0 = pl.multiple_of((step * HP + hh) * D, D)
                ctx_s[base:base + BQ, pl.ds(c0, D)] = o.astype(BF)

    @pl.when(step == NS)
    def _():
        wo_copy.wait()

    @pl.when(step >= NS)
    def _():
        R = S // NO
        r0 = pl.multiple_of((step - NS) * R, R)
        rs = pl.ds(r0, R)
        a = _mm(ctx_s[rs, :], wo_s[...])
        xb = x_ref[rs, :]
        z = jnp.sum((xb * gw_ref[...]).astype(F32), axis=1, keepdims=True)
        g = jax.nn.sigmoid(z)
        b = xb.astype(F32) * b_s[rs, :]
        o_ref[...] = (g * a + (1.0 - g) * b).astype(o_ref.dtype)


@jax.jit
def pallas_gated_mix__compressed_kv_cla__ssm_conv_h3__prompt_kernel(
    A_x, A_c_kv, A_w_q, A_w_uk, A_w_uv, A_w_o, B_q, B_k, B_v, B_shift_k,
    B_ssm_k, B_ssm_D, gate_w,
):
    fwd, inv = _dft_consts()
    per = NS // 8
    hm = lambda s: (0, jnp.minimum(s, NS - 1))
    cm = lambda s: (0, jnp.minimum(s // per, 7))
    full = lambda shape: pl.BlockSpec(shape, lambda s: (0, 0))
    out = pl.pallas_call(
        _kernel,
        grid=(NS + NO,),
        in_specs=[
            full((S, M)), full((S, DC)),
            pl.BlockSpec(memory_space=pl.ANY),
            pl.BlockSpec(memory_space=pl.ANY),
            pl.BlockSpec(memory_space=pl.ANY),
            pl.BlockSpec(memory_space=pl.ANY),
            pl.BlockSpec((S, T), cm), pl.BlockSpec((S, T), cm),
            pl.BlockSpec((4, T), cm),
            pl.BlockSpec((T, S), lambda s: (jnp.minimum(s // per, 7), 0)),
            pl.BlockSpec((1, T), cm),
            full((1, M)), full((2 * T, T)), full((T, 4 * T)),
        ],
        out_specs=pl.BlockSpec((S // NO, M), lambda s: (jnp.maximum(s - NS, 0), 0)),
        out_shape=jax.ShapeDtypeStruct((S, M), A_x.dtype),
        scratch_shapes=[
            pltpu.VMEM((S, H * D), BF), pltpu.VMEM((S, M), F32), pltpu.VMEM((H * D, M), BF),
            pltpu.VMEM((S, T), BF), pltpu.VMEM((NI, 2 * T, T), F32),
            pltpu.VMEM((NI, 2 * T, T), F32), pltpu.VMEM((NI + 1, 2 * T, T), BF),
            pltpu.SemaphoreType.DMA(()),
            pltpu.VMEM((2, M, D), jnp.uint32), pltpu.VMEM((2, DC, D), jnp.uint32),
            pltpu.VMEM((2, DC, D), jnp.uint32), pltpu.SemaphoreType.DMA((3, 2)),
        ],
        compiler_params=pltpu.CompilerParams(
            dimension_semantics=("arbitrary",), vmem_limit_bytes=110 * 1024 * 1024),
    )(A_x[0], A_c_kv[0], A_w_q, A_w_uk,
      A_w_uv, A_w_o.reshape(H * D, M), B_k[0], B_v[0], B_shift_k.T,
      B_ssm_k, B_ssm_D.reshape(1, M), gate_w.reshape(1, M),
      jnp.asarray(fwd, BF), jnp.asarray(inv, BF))
    return out[None]
```
